```python
import os as _os
_os.environ.setdefault("JAX_PLATFORMS", "cpu")
import jax
import jax.numpy as jnp

def _softmax(x, axis=-1):
    return jax.nn.softmax(x, axis=axis)
def _gelu(x):
    return jax.nn.gelu(x, approximate=True)
def _silu(x):
    return jax.nn.silu(x)
def _sigmoid(x):
    return jax.nn.sigmoid(x)
def _layernorm(x, axis=-1, eps=1e-5):
    m = jnp.mean(x, axis=axis, keepdims=True)
    v = jnp.var(x, axis=axis, keepdims=True)
    return (x - m) / jnp.sqrt(v + eps)
def _scatter_add(tgt, idx, src, axis=0):
    return tgt.at[idx].add(src)
def _segment_sum(src, seg, n):
    return jax.ops.segment_sum(src, seg, n)
class _Rng:
    def __init__(self, key):
        self._k = key
    def _next(self):
        self._k, sub = jax.random.split(self._k)
        return sub
    def normal(self, shape):
        return jax.random.normal(self._next(), shape, dtype=jnp.bfloat16)
    def randint(self, lo, hi, shape):
        return jax.random.randint(self._next(), shape, lo, hi, dtype=jnp.int32)
    def uniform(self, shape, lo=0.0, hi=1.0):
        return jax.random.uniform(self._next(), shape, jnp.bfloat16, lo, hi)
    def permutation(self, n):
        return jax.random.permutation(self._next(), n)


kernel_name = 'gated_mix__sliding_local_dilated__moe_arch_mod__prompt'

def setup_inputs():
    _rng = _Rng(jax.random.key(int.from_bytes(__import__("os").urandom(4), "little")))
    _w = (lambda a: (lambda t: t.astype(jnp.bfloat16) if jnp.issubdtype(t.dtype, jnp.floating) else t)(jnp.asarray(a)))
    def _A_setup():
        B, S, D = 1, 2048, 640
        return {
            "x": _w((lambda *s: _rng.normal(s) * 0.05)(B, S, D)),
            "wqkv": _w((lambda *s: _rng.normal(s) * 0.8)(D, 3 * D)),
            "wo": _w((lambda *s: _rng.normal(s) * 0.05)(D, D)),
        }
    _A_in = _A_setup()

    def _B_setup():
        B, S, D, F, C = 1, 2048, 640, 1728, 1
        return {
            "x": _w((lambda *s: _rng.normal(s) * 0.05)(B, S, D)),
            "w_r": _w((lambda *s: _rng.normal(s) * 1.6)(D)),
            "w_gate": _w((lambda *s: _rng.normal(s) * 0.4)(D, F)),
            "w_up": _w((lambda *s: _rng.normal(s) * 0.4)(D, F)),
            "w_down": _w((lambda *s: _rng.normal(s) * 0.4)(F, D)),
        }
    _B_in = _B_setup()

    return {
        "A_x": _A_in["x"],
        "A_wqkv": _A_in["wqkv"],
        "A_wo": _A_in["wo"],
        "B_x": _B_in["x"],
        "B_w_r": _B_in["w_r"],
        "B_w_gate": _B_in["w_gate"],
        "B_w_up": _B_in["w_up"],
        "B_w_down": _B_in["w_down"],
        "gate_w": _w((lambda *s: _rng.normal(s) * 0.05)(640) * 16.0),
    }

def reference(A_x, A_wqkv, A_wo, B_x, B_w_r, B_w_gate, B_w_up, B_w_down, gate_w):
    def _A_ref(x, wqkv, wo):
        B, S, D = x.shape
        H = 32; Dh = D // H
        W, dil = 8, 2
        qkv = (lambda x, *d: x.transpose(*d))((x @ wqkv).reshape(B, S, 3, H, Dh), 2, 0, 3, 1, 4)
        q, k, v = qkv[0], qkv[1], qkv[2]
        scale = Dh ** -0.5
        pos = jnp.arange(S)
        off = jnp.arange(W) * dil
        idx = pos[:, None] - off[None, :]
        mask = idx >= 0
        idx_c = jnp.where(mask, idx, 0).reshape(-1)
        kg = k[:, :, idx_c, :].reshape(B, H, S, W, Dh)
        vg = v[:, :, idx_c, :].reshape(B, H, S, W, Dh)
        logits = jnp.einsum("bhsd,bhswd->bhsw", q, kg) * scale
        logits = jnp.where(mask[None, None, :, :], logits, -1e9)
        attn = _softmax(logits, axis=-1)
        o = jnp.einsum("bhsw,bhswd->bhsd", attn, vg)
        return (lambda x, *d: x.transpose(*d))(o, 0, 2, 1, 3).reshape(B, S, D) @ wo

    def _B_ref(x, w_r, w_gate, w_up, w_down):
        B, S, D = x.shape
        C = 1
        r = x @ w_r
        idx = jnp.argsort(-r, axis=-1)[:, :C]
        idx_e = jnp.repeat(idx.reshape(B, C, 1), D, axis=2)
        x_sel = jnp.take_along_axis(x, idx_e, axis=1)
        g = _silu(x_sel @ w_gate)
        u = x_sel @ w_up
        y = (g * u) @ w_down
        r_sel = _sigmoid(jnp.take_along_axis(r, idx, axis=1))
        y = y * r_sel.reshape(B, C, 1)
        b_off = (jnp.arange(B) * S).reshape(B, 1)
        flat_idx = (idx + b_off).reshape(B * C)
        zero = (x * 0.0).reshape(B * S, D)
        upd = _scatter_add(zero, flat_idx, y.reshape(B * C, D), axis=0)
        return x + upd.reshape(B, S, D)

    x = A_x
    g = _sigmoid((x * gate_w).sum(-1, keepdims=True))
    a = _A_ref(x, A_wqkv, A_wo)
    b = _B_ref(x, B_w_r, B_w_gate, B_w_up, B_w_down)
    return g * a + (1 - g) * b
```

```python
import jax
import jax.numpy as jnp
from jax import lax
import jax.experimental.pallas as pl
import jax.experimental.pallas.tpu as pltpu

S, D, H, DH, F = 2048, 640, 32, 20, 1728
NT = D // 128
W, DIL = 8, 2
HALO = 16
T = 256
NB = S // T
R = 32
DIST = (10, 4, 2, 0, 0)
ORDER = (1, 0, 2, 3)
LOG2E = 1.4426950408889634
QSCALE = (DH ** -0.5) * LOG2E
NEG = -1e9 * LOG2E
F32 = jnp.float32
BF16 = jnp.bfloat16
NT_DIMS = (((1,), (1,)), ((), ()))


def _body(x_hbm, wqkv_hbm, wo_hbm, wr_hbm, gw_hbm, wg_hbm, wu_hbm, wd_hbm, out_hbm,
          x_v, wqkv_v, wt_s, wp_s, wo_v, wop_s, wg_v, wu_v, wd_v, wr_v, gw_v,
          q_s, k_s, v_s, buf, o_s, asel_s, out_v, sem_in, sem_x, sem_out):
    def cp_x(i):
        r0 = i * T if isinstance(i, int) else pl.multiple_of(i * T, T)
        return pltpu.make_async_copy(x_hbm.at[pl.ds(r0, T)], x_v.at[pl.ds(r0, T)], sem_x.at[i])

    def cp_out(i):
        r0 = pl.multiple_of(i * T, T)
        return pltpu.make_async_copy(out_v.at[pl.ds(r0, T)], out_hbm.at[pl.ds(r0, T)], sem_out.at[i])

    cp_w = [pltpu.make_async_copy(wqkv_hbm.at[:, pl.ds(c * D, D)], wqkv_v.at[c], sem_in.at[c])
            for c in range(3)]
    cp_wo = pltpu.make_async_copy(wo_hbm, wo_v, sem_in.at[3])
    cp_wg = pltpu.make_async_copy(wg_hbm, wg_v, sem_in.at[4])
    cp_wu = pltpu.make_async_copy(wu_hbm, wu_v, sem_in.at[5])
    cp_wd = pltpu.make_async_copy(wd_hbm, wd_v, sem_in.at[6])
    cp_wr = pltpu.make_async_copy(wr_hbm, wr_v, sem_in.at[7])
    cp_gw = pltpu.make_async_copy(gw_hbm, gw_v, sem_in.at[8])
    cp_x(0).start()
    cp_w[1].start()

    def permute_w(c, b):
        for kt in range(NT):
            wt = wqkv_v[c, kt * 128:(kt + 1) * 128, :].T
            wt_s[b, kt] = pltpu.bitcast(wt, jnp.uint32)
        for kt in range(NT):
            for dd in range(DH // 2):
                wp_s[c, dd * 32:(dd + 1) * 32, kt * 128:(kt + 1) * 128] = (
                    wt_s[b, kt, pl.ds(dd, H, stride=DH // 2), :])

    def permute_wo(b):
        for nt in range(NT):
            wt_s[b, nt] = pltpu.bitcast(wo_v[:, nt * 128:(nt + 1) * 128], jnp.uint32)
        for nt in range(NT):
            for dd in range(DH // 2):
                wop_s[dd * 32:(dd + 1) * 32, nt * 128:(nt + 1) * 128] = (
                    wt_s[b, nt, pl.ds(dd, H, stride=DH // 2), :])

    TH = T // 2
    obuf = o_s

    def xrows(i):
        return pl.ds(pl.multiple_of(T + i * TH, TH), TH)

    def stage_x(i):
        r0 = pl.multiple_of(i * T, T)
        buf[xrows(i), :] = pltpu.bitcast(x_v[pl.ds(r0, T), :], jnp.uint32)

    def proj(i, c):
        r0 = pl.multiple_of(i * T, T)
        xb = pltpu.bitcast(buf[xrows(i), :], BF16)
        y = lax.dot_general(xb, pltpu.bitcast(wp_s[c], BF16), NT_DIMS, preferred_element_type=F32)
        for j in range(NT):
            yj = y[:, j * 128:(j + 1) * 128]
            if c == 0:
                q_s[i % 2, j] = yj * QSCALE
            elif c == 1:
                k_s[j, pl.ds(r0 + HALO, T), :] = yj
            else:
                v_s[j, pl.ds(r0 + HALO, T), :] = yj

    def router(i, carry):
        bv, bi = carry
        r0 = pl.multiple_of(i * T, T)
        xf = pltpu.bitcast(buf[xrows(i), :], BF16).astype(F32)
        r = jnp.sum(xf * wr, axis=-1, keepdims=True).astype(BF16).astype(F32)
        ids = lax.broadcasted_iota(jnp.int32, (8, 1), 0) + r0
        for c in range(T // 8):
            rc = r[c * 8:(c + 1) * 8]
            upd = rc > bv
            bv = jnp.where(upd, rc, bv)
            bi = jnp.where(upd, ids + c * 8, bi)
        return bv, bi

    lane = lax.broadcasted_iota(jnp.int32, (R, 128), 1)
    odd = (lane & 1) == 1
    row = lax.broadcasted_iota(jnp.int32, (R, 128), 0)

    def attn(i, c):
        r0 = pl.multiple_of(i * T, T)
        q = [q_s[i % 2, j, c * R:(c + 1) * R, :] for j in range(NT)]
        ls = [None] * W
        HW = W // 2
        for sft in range(HW):
            st = r0 + (HALO + c * R - DIL * sft - 8)
            ta = tb = None
            for j in range(NT):
                ke = k_s[j, pl.ds(st, R + 8), :]
                pa = q[j] * ke[8:]
                pb = q[j] * ke[:R]
                ta = pa if ta is None else ta + pa
                tb = pb if tb is None else tb + pb
            for w, t in ((sft, ta), (sft + HW, tb)):
                t = t + pltpu.roll(t, 64, 1)
                u = t + pltpu.roll(t, 1, 1)
                l = jnp.where(odd, u, pltpu.roll(u, 127, 1))
                if c * R < DIL * w:
                    l = jnp.where(row + (r0 + c * R) >= DIL * w, l, NEG)
                ls[w] = l
        m = ls[0]
        for w in range(1, W):
            m = jnp.maximum(m, ls[w])
        ps = [jnp.exp2(l - m) for l in ls]
        den = ps[0]
        for w in range(1, W):
            den = den + ps[w]
        inv = 1.0 / den
        res = []
        for j in range(NT):
            acc = None
            for sft in range(HW):
                st = r0 + (HALO + c * R - DIL * sft - 8)
                ve = v_s[j, pl.ds(st, R + 8), :]
                term = ps[sft] * ve[8:] + ps[sft + HW] * ve[:R]
                acc = term if acc is None else acc + term
            res.append(pltpu.bitcast((acc * inv).astype(BF16), jnp.uint32))

        for j in range(NT):
            obuf[pl.ds(pl.multiple_of((i % 2) * TH + c * (R // 2), R // 2), R // 2),
                 j * 128:(j + 1) * 128] = res[j]

    def outproj(i, lo, n, ix):
        r0 = pl.multiple_of(i * T, T)
        ob = pltpu.bitcast(obuf[pl.ds(pl.multiple_of((i % 2) * TH + lo // 2, 8), n // 2), :], BF16)
        a = jnp.dot(ob, pltpu.bitcast(wop_s[...], BF16), preferred_element_type=F32)
        asel_s[pl.ds(r0 + lo, n), :] = a
        xf = pltpu.bitcast(buf[pl.ds(pl.multiple_of(T + ix * TH + lo // 2, 8), n // 2), :], BF16).astype(F32)
        g = jax.nn.sigmoid(jnp.sum(xf * gw, axis=-1, keepdims=True))
        out_v[pl.ds(r0 + lo, n), :] = (g * a + (1.0 - g) * xf).astype(BF16)

    cp_x(0).wait()
    cp_w[0].start()
    cp_wr.start()
    cp_gw.start()
    stage_x(0)
    cp_w[1].wait()
    cp_w[2].start()
    cp_x(1).start()
    permute_w(1, 0)
    proj(0, 1)
    cp_w[0].wait()
    cp_wo.start()
    permute_w(0, 1)
    cp_w[2].wait()
    for i in range(2, NB):
        cp_x(i).start()
    proj(0, 0)
    permute_w(2, 0)
    cp_wo.wait()
    cp_wr.wait()
    cp_gw.wait()
    proj(0, 2)
    permute_wo(1)
    wr = wr_v[...].astype(F32).reshape(1, D)
    gw = gw_v[...].astype(F32).reshape(1, D)
    carry = router(0, (jnp.full((8, 1), -jnp.inf, F32), jnp.zeros((8, 1), jnp.int32)))
    for j in range(NT):
        k_s[j, 0:HALO, :] = jnp.zeros((HALO, 128), F32)
        v_s[j, 0:HALO, :] = jnp.broadcast_to(v_s[j, HALO:HALO + 1, :], (HALO, 128))

    NC = T // R
    obuf[TH:T, :] = jnp.zeros((TH, D), jnp.uint32)

    def loop(i, carry):
        cp_x(i + 1).wait()
        ip = jnp.where(i == 0, NB - 1, i - 1)
        ix = jnp.maximum(i - 1, 0)
        stage_x(i + 1)
        done = 0
        for p, c in enumerate(ORDER + (None,)):
            for cc in range(done, done + DIST[p] * NC // 16):
                attn(i, cc)
            done += DIST[p] * NC // 16
            if c == 3:
                outproj(ip, 0, T, ix)
            elif c is not None:
                proj(i + 1, c)
        assert done == NC
        carry = router(i + 1, carry)

        @pl.when(i > 0)
        def _():
            cp_out(i - 1).start()

        @pl.when(i == 1)
        def _():
            cp_wg.start()
            cp_wu.start()
            cp_wd.start()
        return carry

    bv, bi = lax.fori_loop(0, NB - 1, loop, carry)
    rmax = jnp.max(bv, axis=0, keepdims=True)
    idx = jnp.min(jnp.where(bv == rmax, bi, S))
    idx = jnp.clip(idx, 0, S - 1)

    cp_wg.wait()
    cp_wu.wait()
    cp_wd.wait()
    t0 = pl.multiple_of((idx // 16) * 16, 16)
    xt = x_v[pl.ds(t0, 16), :]
    last = NB - 1
    for c in range(0, 2):
        attn(last, c)
    outproj(last - 1, 0, T, last - 1)
    cp_out(last - 1).start()
    for c in range(2, 4):
        attn(last, c)
    gg = lax.dot_general(xt, wg_v[...], NT_DIMS, preferred_element_type=F32)
    outproj(last, 0, T // 2, last)
    uu = lax.dot_general(xt, wu_v[...], NT_DIMS, preferred_element_type=F32)
    for c in range(4, NC):
        attn(last, c)
    hh = (gg * jax.nn.sigmoid(gg) * uu).astype(BF16)
    y = jnp.dot(hh, wd_v[...], preferred_element_type=F32)
    outproj(last, T // 2, T // 2, last)
    xf = xt.astype(F32)
    g = jax.nn.sigmoid(jnp.sum(xf * gw, axis=-1, keepdims=True))
    new = g * asel_s[pl.ds(t0, 16), :] + (1.0 - g) * (xf + y * jax.nn.sigmoid(rmax))
    for i in range(NB - 1):
        cp_out(i).wait()
    rows = lax.broadcasted_iota(jnp.int32, (16, D), 0) + t0
    out_v[pl.ds(t0, 16), :] = jnp.where(rows == idx, new.astype(BF16), out_v[pl.ds(t0, 16), :])
    cp_out(NB - 1).start()

    @pl.when(idx < S - T)
    def _():
        cp = pltpu.make_async_copy(out_v.at[pl.ds(t0, 16)], out_hbm.at[pl.ds(t0, 16)], sem_out.at[0])
        cp.start()
        cp.wait()

    cp_out(NB - 1).wait()


def _call(x, wqkv, wo, wr, gw, wg, wu, wd):
    hbm = pl.BlockSpec(memory_space=pltpu.MemorySpace.HBM)
    return pl.pallas_call(
        _body,
        out_shape=jax.ShapeDtypeStruct((S, D), BF16),
        in_specs=[hbm] * 8,
        out_specs=hbm,
        scratch_shapes=[
            pltpu.VMEM((S, D), BF16),
            pltpu.VMEM((3, D, D), BF16),
            pltpu.VMEM((2, NT, D // 2, 128), jnp.uint32),
            pltpu.VMEM((3, D // 2, D), jnp.uint32),
            pltpu.VMEM((D, D), BF16),
            pltpu.VMEM((D // 2, D), jnp.uint32),
            pltpu.VMEM((F, D), BF16),
            pltpu.VMEM((F, D), BF16),
            pltpu.VMEM((F, D), BF16),
            pltpu.VMEM((D,), BF16),
            pltpu.VMEM((D,), BF16),
            pltpu.VMEM((2, NT, T, 128), F32),
            pltpu.VMEM((NT, S + HALO, 128), F32),
            pltpu.VMEM((NT, S + HALO, 128), F32),
            pltpu.VMEM((T + S // 2, D), jnp.uint32),
            pltpu.VMEM((T, D), jnp.uint32),
            pltpu.VMEM((S, D), F32),
            pltpu.VMEM((S, D), BF16),
            pltpu.SemaphoreType.DMA((9,)),
            pltpu.SemaphoreType.DMA((NB,)),
            pltpu.SemaphoreType.DMA((NB,)),
        ],
        compiler_params=pltpu.CompilerParams(vmem_limit_bytes=100 * 1024 * 1024),
    )(x, wqkv, wo, wr, gw, wg, wu, wd)


@jax.jit
def pallas_gated_mix__sliding_local_dilated__moe_arch_mod__prompt_kernel(
        A_x, A_wqkv, A_wo, B_x, B_w_r, B_w_gate, B_w_up, B_w_down, gate_w):
    out = _call(A_x.reshape(S, D), A_wqkv, A_wo, B_w_r, gate_w,
                B_w_gate.T, B_w_up.T, B_w_down)
    return out.reshape(1, S, D)
```

```python
import jax
import jax.numpy as jnp
from jax import lax
import jax.experimental.pallas as pl
import jax.experimental.pallas.tpu as pltpu

S, D, H, DH, F = 2048, 640, 32, 20, 1728
NT = D // 128
W, DIL = 8, 2
HALO = 16
T = 256
NB = S // T
R = 32
DIST = (16, 0, 0, 0, 0)
ORDER = (2, 1, 0, 3)
LOG2E = 1.4426950408889634
QSCALE = (DH ** -0.5) * LOG2E
NEG = -1e9 * LOG2E
F32 = jnp.float32
BF16 = jnp.bfloat16
NT_DIMS = (((1,), (1,)), ((), ()))


def _body(x_hbm, wqkv_hbm, wo_hbm, wr_hbm, gw_hbm, wg_hbm, wu_hbm, wd_hbm, out_hbm,
          x_v, wqkv_v, wt_s, wp_s, wo_v, wop_s, wg_v, wu_v, wd_v, wr_v, gw_v,
          q_s, k_s, v_s, buf, o_s, asel_s, out_v, sem_in, sem_x, sem_out):
    def cp_x(i):
        r0 = i * T if isinstance(i, int) else pl.multiple_of(i * T, T)
        return pltpu.make_async_copy(x_hbm.at[pl.ds(r0, T)], x_v.at[pl.ds(r0, T)], sem_x.at[i])

    def cp_out(i):
        r0 = pl.multiple_of(i * T, T)
        return pltpu.make_async_copy(out_v.at[pl.ds(r0, T)], out_hbm.at[pl.ds(r0, T)], sem_out.at[i])

    cp_w = [pltpu.make_async_copy(wqkv_hbm.at[:, pl.ds(c * D, D)], wqkv_v.at[c], sem_in.at[c])
            for c in range(3)]
    cp_wo = pltpu.make_async_copy(wo_hbm, wo_v, sem_in.at[3])
    cp_wg = pltpu.make_async_copy(wg_hbm, wg_v, sem_in.at[4])
    cp_wu = pltpu.make_async_copy(wu_hbm, wu_v, sem_in.at[5])
    cp_wd = pltpu.make_async_copy(wd_hbm, wd_v, sem_in.at[6])
    cp_wr = pltpu.make_async_copy(wr_hbm, wr_v, sem_in.at[7])
    cp_gw = pltpu.make_async_copy(gw_hbm, gw_v, sem_in.at[8])
    cp_x(0).start()
    cp_w[1].start()

    def permute_w(c, b):
        for kt in range(NT):
            wt = wqkv_v[c, kt * 128:(kt + 1) * 128, :].T
            wt_s[b, kt] = pltpu.bitcast(wt, jnp.uint32)
        for kt in range(NT):
            for dd in range(DH // 2):
                wp_s[c, dd * 32:(dd + 1) * 32, kt * 128:(kt + 1) * 128] = (
                    wt_s[b, kt, pl.ds(dd, H, stride=DH // 2), :])

    def permute_wo(b):
        for nt in range(NT):
            wt_s[b, nt] = pltpu.bitcast(wo_v[:, nt * 128:(nt + 1) * 128], jnp.uint32)
        for nt in range(NT):
            for dd in range(DH // 2):
                wop_s[dd * 32:(dd + 1) * 32, nt * 128:(nt + 1) * 128] = (
                    wt_s[b, nt, pl.ds(dd, H, stride=DH // 2), :])

    TH = T // 2
    obuf = o_s

    def xrows(i):
        return pl.ds(pl.multiple_of(T + i * TH, TH), TH)

    def stage_x(i):
        r0 = pl.multiple_of(i * T, T)
        buf[xrows(i), :] = pltpu.bitcast(x_v[pl.ds(r0, T), :], jnp.uint32)

    def proj(i, c):
        r0 = pl.multiple_of(i * T, T)
        xb = pltpu.bitcast(buf[xrows(i), :], BF16)
        y = lax.dot_general(xb, pltpu.bitcast(wp_s[c], BF16), NT_DIMS, preferred_element_type=F32)
        for j in range(NT):
            yj = y[:, j * 128:(j + 1) * 128]
            if c == 0:
                q_s[i % 2, j] = yj * QSCALE
            elif c == 1:
                k_s[j, pl.ds(r0 + HALO, T), :] = yj
            else:
                v_s[j, pl.ds(r0 + HALO, T), :] = yj

    def router(i, carry):
        bv, bi = carry
        r0 = pl.multiple_of(i * T, T)
        xf = pltpu.bitcast(buf[xrows(i), :], BF16).astype(F32)
        r = jnp.sum(xf * wr, axis=-1, keepdims=True).astype(BF16).astype(F32)
        ids = lax.broadcasted_iota(jnp.int32, (8, 1), 0) + r0
        for c in range(T // 8):
            rc = r[c * 8:(c + 1) * 8]
            upd = rc > bv
            bv = jnp.where(upd, rc, bv)
            bi = jnp.where(upd, ids + c * 8, bi)
        return bv, bi

    lane = lax.broadcasted_iota(jnp.int32, (R, 128), 1)
    odd = (lane & 1) == 1
    row = lax.broadcasted_iota(jnp.int32, (R, 128), 0)

    def attn(i, c):
        r0 = pl.multiple_of(i * T, T)
        q = [q_s[i % 2, j, c * R:(c + 1) * R, :] for j in range(NT)]
        ls = [None] * W
        HW = W // 2
        for sft in range(HW):
            st = r0 + (HALO + c * R - DIL * sft - 8)
            ta = tb = None
            for j in range(NT):
                ke = k_s[j, pl.ds(st, R + 8), :]
                pa = q[j] * ke[8:]
                pb = q[j] * ke[:R]
                ta = pa if ta is None else ta + pa
                tb = pb if tb is None else tb + pb
            for w, t in ((sft, ta), (sft + HW, tb)):
                t = t + pltpu.roll(t, 64, 1)
                u = t + pltpu.roll(t, 1, 1)
                l = jnp.where(odd, u, pltpu.roll(u, 127, 1))
                if c * R < DIL * w:
                    l = jnp.where(row + (r0 + c * R) >= DIL * w, l, NEG)
                ls[w] = l
        m = ls[0]
        for w in range(1, W):
            m = jnp.maximum(m, ls[w])
        ps = [jnp.exp2(l - m) for l in ls]
        den = ps[0]
        for w in range(1, W):
            den = den + ps[w]
        inv = 1.0 / den
        res = []
        for j in range(NT):
            acc = None
            for sft in range(HW):
                st = r0 + (HALO + c * R - DIL * sft - 8)
                ve = v_s[j, pl.ds(st, R + 8), :]
                acc = ps[sft] * ve[8:] if acc is None else acc + ps[sft] * ve[8:]
                acc = acc + ps[sft + HW] * ve[:R]
            res.append(pltpu.bitcast((acc * inv).astype(BF16), jnp.uint32))

        for j in range(NT):
            obuf[pl.ds(pl.multiple_of((i % 2) * TH + c * (R // 2), R // 2), R // 2),
                 j * 128:(j + 1) * 128] = res[j]

    def outproj(i, lo, n):
        r0 = pl.multiple_of(i * T, T)
        ob = pltpu.bitcast(obuf[pl.ds(pl.multiple_of((i % 2) * TH + lo // 2, 8), n // 2), :], BF16)
        a = jnp.dot(ob, pltpu.bitcast(wop_s[...], BF16), preferred_element_type=F32)
        asel_s[pl.ds(r0 + lo, n), :] = a
        xf = pltpu.bitcast(buf[pl.ds(pl.multiple_of(T + i * TH + lo // 2, 8), n // 2), :], BF16).astype(F32)
        g = jax.nn.sigmoid(jnp.sum(xf * gw, axis=-1, keepdims=True))
        out_v[pl.ds(r0 + lo, n), :] = (g * a + (1.0 - g) * xf).astype(BF16)

    cp_x(0).wait()
    cp_w[0].start()
    cp_wr.start()
    cp_gw.start()
    stage_x(0)
    cp_w[1].wait()
    cp_w[2].start()
    cp_x(1).start()
    permute_w(1, 0)
    proj(0, 1)
    cp_w[0].wait()
    cp_wo.start()
    permute_w(0, 1)
    cp_w[2].wait()
    for i in range(2, NB):
        cp_x(i).start()
    proj(0, 0)
    permute_w(2, 0)
    cp_wo.wait()
    cp_wr.wait()
    cp_gw.wait()
    proj(0, 2)
    permute_wo(1)
    wr = wr_v[...].astype(F32).reshape(1, D)
    gw = gw_v[...].astype(F32).reshape(1, D)
    carry = router(0, (jnp.full((8, 1), -jnp.inf, F32), jnp.zeros((8, 1), jnp.int32)))
    for j in range(NT):
        k_s[j, 0:HALO, :] = jnp.zeros((HALO, 128), F32)
        v_s[j, 0:HALO, :] = jnp.broadcast_to(v_s[j, HALO:HALO + 1, :], (HALO, 128))

    NC = T // R

    def loop(i, carry):
        cp_x(i + 1).wait()
        stage_x(i + 1)
        done = 0
        for p, c in enumerate(ORDER + (None,)):
            for cc in range(done, done + DIST[p] * NC // 16):
                attn(i, cc)
            done += DIST[p] * NC // 16
            if c == 3:
                outproj(i, 0, T)
            elif c is not None:
                proj(i + 1, c)
        assert done == NC
        carry = router(i + 1, carry)

        cp_out(i).start()

        @pl.when(i == 1)
        def _():
            cp_wg.start()
            cp_wu.start()
            cp_wd.start()
        return carry

    bv, bi = lax.fori_loop(0, NB - 1, loop, carry)
    rmax = jnp.max(bv, axis=0, keepdims=True)
    idx = jnp.min(jnp.where(bv == rmax, bi, S))
    idx = jnp.clip(idx, 0, S - 1)

    cp_wg.wait()
    cp_wu.wait()
    cp_wd.wait()
    t0 = pl.multiple_of((idx // 16) * 16, 16)
    xt = x_v[pl.ds(t0, 16), :]
    last = NB - 1
    for c in range(0, NC // 2):
        attn(last, c)
    gg = lax.dot_general(xt, wg_v[...], NT_DIMS, preferred_element_type=F32)
    outproj(last, 0, T // 2)
    for c in range(NC // 2, NC):
        attn(last, c)
    uu = lax.dot_general(xt, wu_v[...], NT_DIMS, preferred_element_type=F32)
    outproj(last, T // 2, T // 2)
    hh = (gg * jax.nn.sigmoid(gg) * uu).astype(BF16)
    y = jnp.dot(hh, wd_v[...], preferred_element_type=F32)
    xf = xt.astype(F32)
    g = jax.nn.sigmoid(jnp.sum(xf * gw, axis=-1, keepdims=True))
    new = g * asel_s[pl.ds(t0, 16), :] + (1.0 - g) * (xf + y * jax.nn.sigmoid(rmax))
    for i in range(NB - 1):
        cp_out(i).wait()
    rows = lax.broadcasted_iota(jnp.int32, (16, D), 0) + t0
    out_v[pl.ds(t0, 16), :] = jnp.where(rows == idx, new.astype(BF16), out_v[pl.ds(t0, 16), :])
    cp_out(NB - 1).start()

    @pl.when(idx < S - T)
    def _():
        cp = pltpu.make_async_copy(out_v.at[pl.ds(t0, 16)], out_hbm.at[pl.ds(t0, 16)], sem_out.at[0])
        cp.start()
        cp.wait()

    cp_out(NB - 1).wait()


def _call(x, wqkv, wo, wr, gw, wg, wu, wd):
    hbm = pl.BlockSpec(memory_space=pltpu.MemorySpace.HBM)
    return pl.pallas_call(
        _body,
        out_shape=jax.ShapeDtypeStruct((S, D), BF16),
        in_specs=[hbm] * 8,
        out_specs=hbm,
        scratch_shapes=[
            pltpu.VMEM((S, D), BF16),
            pltpu.VMEM((3, D, D), BF16),
            pltpu.VMEM((2, NT, D // 2, 128), jnp.uint32),
            pltpu.VMEM((3, D // 2, D), jnp.uint32),
            pltpu.VMEM((D, D), BF16),
            pltpu.VMEM((D // 2, D), jnp.uint32),
            pltpu.VMEM((F, D), BF16),
            pltpu.VMEM((F, D), BF16),
            pltpu.VMEM((F, D), BF16),
            pltpu.VMEM((D,), BF16),
            pltpu.VMEM((D,), BF16),
            pltpu.VMEM((2, NT, T, 128), F32),
            pltpu.VMEM((NT, S + HALO, 128), F32),
            pltpu.VMEM((NT, S + HALO, 128), F32),
            pltpu.VMEM((T + S // 2, D), jnp.uint32),
            pltpu.VMEM((T, D), jnp.uint32),
            pltpu.VMEM((S, D), F32),
            pltpu.VMEM((S, D), BF16),
            pltpu.SemaphoreType.DMA((9,)),
            pltpu.SemaphoreType.DMA((NB,)),
            pltpu.SemaphoreType.DMA((NB,)),
        ],
        compiler_params=pltpu.CompilerParams(
            vmem_limit_bytes=100 * 1024 * 1024,
            flags={"XLA_TPU_EVENLY_DISTRIBUTE_CRITICAL_NODES": True}),
    )(x, wqkv, wo, wr, gw, wg, wu, wd)


@jax.jit
def pallas_gated_mix__sliding_local_dilated__moe_arch_mod__prompt_kernel(
        A_x, A_wqkv, A_wo, B_x, B_w_r, B_w_gate, B_w_up, B_w_down, gate_w):
    out = _call(A_x.reshape(S, D), A_wqkv, A_wo, B_w_r, gate_w,
                B_w_gate.T, B_w_up.T, B_w_down)
    return out.reshape(1, S, D)
```

```python
import jax
import jax.numpy as jnp
from jax import lax
import jax.experimental.pallas as pl
import jax.experimental.pallas.tpu as pltpu

S, D, H, DH, F = 2048, 640, 32, 20, 1728
NT = D // 128
W, DIL = 8, 2
HALO = 16
T = 256
NB = S // T
R = 32
DIST = (16, 0, 0, 0, 0)
ORDER = (2, 1, 0, 3)
LOG2E = 1.4426950408889634
QSCALE = (DH ** -0.5) * LOG2E
NEG = -1e9 * LOG2E
F32 = jnp.float32
BF16 = jnp.bfloat16
NT_DIMS = (((1,), (1,)), ((), ()))


def _body(x_hbm, wqkv_hbm, wo_hbm, wr_hbm, gw_hbm, wg_hbm, wu_hbm, wd_hbm, out_hbm,
          x_v, wqkv_v, wt_s, wp_s, wo_v, wop_s, wg_v, wu_v, wd_v, wr_v, gw_v,
          q_s, k_s, v_s, buf, o_s, asel_s, out_v, sem_in, sem_x, sem_out, sem_tail):
    def cp_x(i):
        r0 = i * T if isinstance(i, int) else pl.multiple_of(i * T, T)
        return pltpu.make_async_copy(x_hbm.at[pl.ds(r0, T)], x_v.at[pl.ds(r0, T)], sem_x.at[i])

    def cp_out(i):
        r0 = pl.multiple_of(i * T, T)
        return pltpu.make_async_copy(out_v.at[pl.ds(r0, T)], out_hbm.at[pl.ds(r0, T)], sem_out.at[i])

    cp_w = [pltpu.make_async_copy(wqkv_hbm.at[:, pl.ds(c * D, D)], wqkv_v.at[c], sem_in.at[c])
            for c in range(3)]
    cp_wo = pltpu.make_async_copy(wo_hbm, wo_v, sem_in.at[3])
    cp_wg = pltpu.make_async_copy(wg_hbm, wg_v, sem_in.at[4])
    cp_wu = pltpu.make_async_copy(wu_hbm, wu_v, sem_in.at[5])
    cp_wd = pltpu.make_async_copy(wd_hbm, wd_v, sem_in.at[6])
    cp_wr = pltpu.make_async_copy(wr_hbm, wr_v, sem_in.at[7])
    cp_gw = pltpu.make_async_copy(gw_hbm, gw_v, sem_in.at[8])
    cp_x(0).start()
    cp_w[1].start()

    def permute_w(c, b):
        for kt in range(NT):
            wt = wqkv_v[c, kt * 128:(kt + 1) * 128, :].T
            wt_s[b, kt] = pltpu.bitcast(wt, jnp.uint32)
        for kt in range(NT):
            for dd in range(DH // 2):
                wp_s[c, dd * 32:(dd + 1) * 32, kt * 128:(kt + 1) * 128] = (
                    wt_s[b, kt, pl.ds(dd, H, stride=DH // 2), :])

    def permute_wo(b):
        for nt in range(NT):
            wt_s[b, nt] = pltpu.bitcast(wo_v[:, nt * 128:(nt + 1) * 128], jnp.uint32)
        for nt in range(NT):
            for dd in range(DH // 2):
                wop_s[dd * 32:(dd + 1) * 32, nt * 128:(nt + 1) * 128] = (
                    wt_s[b, nt, pl.ds(dd, H, stride=DH // 2), :])

    TH = T // 2
    obuf = o_s

    def xrows(i):
        return pl.ds(pl.multiple_of(T + i * TH, TH), TH)

    def stage_x(i):
        r0 = pl.multiple_of(i * T, T)
        buf[xrows(i), :] = pltpu.bitcast(x_v[pl.ds(r0, T), :], jnp.uint32)

    def proj(i, c):
        r0 = pl.multiple_of(i * T, T)
        xb = pltpu.bitcast(buf[xrows(i), :], BF16)
        y = lax.dot_general(xb, pltpu.bitcast(wp_s[c], BF16), NT_DIMS, preferred_element_type=F32)
        for j in range(NT):
            yj = y[:, j * 128:(j + 1) * 128]
            if c == 0:
                q_s[i % 2, j] = yj * QSCALE
            elif c == 1:
                k_s[j, pl.ds(r0 + HALO, T), :] = yj
            else:
                v_s[j, pl.ds(r0 + HALO, T), :] = yj

    def router(i, carry):
        bv, bi = carry
        r0 = pl.multiple_of(i * T, T)
        xf = pltpu.bitcast(buf[xrows(i), :], BF16).astype(F32)
        r = jnp.sum(xf * wr, axis=-1, keepdims=True).astype(BF16).astype(F32)
        ids = lax.broadcasted_iota(jnp.int32, (8, 1), 0) + r0
        for c in range(T // 8):
            rc = r[c * 8:(c + 1) * 8]
            upd = rc > bv
            bv = jnp.where(upd, rc, bv)
            bi = jnp.where(upd, ids + c * 8, bi)
        return bv, bi

    lane = lax.broadcasted_iota(jnp.int32, (R, 128), 1)
    odd = (lane & 1) == 1
    row = lax.broadcasted_iota(jnp.int32, (R, 128), 0)

    def attn(i, c):
        r0 = pl.multiple_of(i * T, T)
        q = [q_s[i % 2, j, c * R:(c + 1) * R, :] for j in range(NT)]
        ls = [None] * W
        HW = W // 2
        for sft in range(HW):
            st = r0 + (HALO + c * R - DIL * sft - 8)
            ta = tb = None
            for j in range(NT):
                ke = k_s[j, pl.ds(st, R + 8), :]
                pa = q[j] * ke[8:]
                pb = q[j] * ke[:R]
                ta = pa if ta is None else ta + pa
                tb = pb if tb is None else tb + pb
            for w, t in ((sft, ta), (sft + HW, tb)):
                t = t + pltpu.roll(t, 64, 1)
                u = t + pltpu.roll(t, 1, 1)
                l = jnp.where(odd, u, pltpu.roll(u, 127, 1))
                if c * R < DIL * w:
                    l = jnp.where(row + (r0 + c * R) >= DIL * w, l, NEG)
                ls[w] = l
        m = ls[0]
        for w in range(1, W):
            m = jnp.maximum(m, ls[w])
        ps = [jnp.exp2(l - m) for l in ls]
        den = ps[0]
        for w in range(1, W):
            den = den + ps[w]
        inv = 1.0 / den
        res = []
        for j in range(NT):
            acc = None
            for sft in range(HW):
                st = r0 + (HALO + c * R - DIL * sft - 8)
                ve = v_s[j, pl.ds(st, R + 8), :]
                acc = ps[sft] * ve[8:] if acc is None else acc + ps[sft] * ve[8:]
                acc = acc + ps[sft + HW] * ve[:R]
            res.append(pltpu.bitcast((acc * inv).astype(BF16), jnp.uint32))

        for j in range(NT):
            obuf[pl.ds(pl.multiple_of((i % 2) * TH + c * (R // 2), R // 2), R // 2),
                 j * 128:(j + 1) * 128] = res[j]

    def outproj(i, lo, n):
        r0 = pl.multiple_of(i * T, T)
        ob = pltpu.bitcast(obuf[pl.ds(pl.multiple_of((i % 2) * TH + lo // 2, 8), n // 2), :], BF16)
        a = jnp.dot(ob, pltpu.bitcast(wop_s[...], BF16), preferred_element_type=F32)
        asel_s[pl.ds(r0 + lo, n), :] = a
        xf = pltpu.bitcast(buf[pl.ds(pl.multiple_of(T + i * TH + lo // 2, 8), n // 2), :], BF16).astype(F32)
        g = jax.nn.sigmoid(jnp.sum(xf * gw, axis=-1, keepdims=True))
        out_v[pl.ds(r0 + lo, n), :] = (g * a + (1.0 - g) * xf).astype(BF16)

    cp_x(0).wait()
    cp_w[0].start()
    cp_wr.start()
    cp_gw.start()
    stage_x(0)
    cp_w[1].wait()
    cp_w[2].start()
    cp_x(1).start()
    permute_w(1, 0)
    proj(0, 1)
    cp_w[0].wait()
    cp_wo.start()
    permute_w(0, 1)
    cp_w[2].wait()
    for i in range(2, NB):
        cp_x(i).start()
    proj(0, 0)
    permute_w(2, 0)
    cp_wo.wait()
    cp_wr.wait()
    cp_gw.wait()
    proj(0, 2)
    permute_wo(1)
    wr = wr_v[...].astype(F32).reshape(1, D)
    gw = gw_v[...].astype(F32).reshape(1, D)
    carry = router(0, (jnp.full((8, 1), -jnp.inf, F32), jnp.zeros((8, 1), jnp.int32)))
    for j in range(NT):
        k_s[j, 0:HALO, :] = jnp.zeros((HALO, 128), F32)
        v_s[j, 0:HALO, :] = jnp.broadcast_to(v_s[j, HALO:HALO + 1, :], (HALO, 128))

    NC = T // R

    def loop(i, carry):
        cp_x(i + 1).wait()
        stage_x(i + 1)
        done = 0
        for p, c in enumerate(ORDER + (None,)):
            for cc in range(done, done + DIST[p] * NC // 16):
                attn(i, cc)
            done += DIST[p] * NC // 16
            if c == 3:
                outproj(i, 0, T)
            elif c is not None:
                proj(i + 1, c)
        assert done == NC
        carry = router(i + 1, carry)

        cp_out(i).start()

        @pl.when(i == 1)
        def _():
            cp_wg.start()
            cp_wu.start()
            cp_wd.start()
        return carry

    bv, bi = lax.fori_loop(0, NB - 1, loop, carry)
    rmax = jnp.max(bv, axis=0, keepdims=True)
    idx = jnp.min(jnp.where(bv == rmax, bi, S))
    idx = jnp.clip(idx, 0, S - 1)

    cp_wg.wait()
    cp_wu.wait()
    cp_wd.wait()
    t0 = pl.multiple_of((idx // 16) * 16, 16)
    xt = x_v[pl.ds(t0, 16), :]
    last = NB - 1
    for c in range(0, NC // 2):
        attn(last, c)
    gg = lax.dot_general(xt, wg_v[...], NT_DIMS, preferred_element_type=F32)
    outproj(last, 0, T // 2)
    cp_h = [pltpu.make_async_copy(out_v.at[pl.ds(S - T + e * TH, TH)], out_hbm.at[pl.ds(S - T + e * TH, TH)],
                                  sem_tail.at[e]) for e in range(2)]
    cp_h[0].start()
    for c in range(NC // 2, NC):
        attn(last, c)
    uu = lax.dot_general(xt, wu_v[...], NT_DIMS, preferred_element_type=F32)
    outproj(last, T // 2, T // 2)
    hh = (gg * jax.nn.sigmoid(gg) * uu).astype(BF16)
    y = jnp.dot(hh, wd_v[...], preferred_element_type=F32)
    xf = xt.astype(F32)
    g = jax.nn.sigmoid(jnp.sum(xf * gw, axis=-1, keepdims=True))
    new = g * asel_s[pl.ds(t0, 16), :] + (1.0 - g) * (xf + y * jax.nn.sigmoid(rmax))
    for i in range(NB - 1):
        cp_out(i).wait()
    cp_h[0].wait()
    rows = lax.broadcasted_iota(jnp.int32, (16, D), 0) + t0
    out_v[pl.ds(t0, 16), :] = jnp.where(rows == idx, new.astype(BF16), out_v[pl.ds(t0, 16), :])
    cp_h[1].start()

    @pl.when(idx < S - TH)
    def _():
        cp = pltpu.make_async_copy(out_v.at[pl.ds(t0, 16)], out_hbm.at[pl.ds(t0, 16)], sem_out.at[0])
        cp.start()
        cp.wait()

    cp_h[1].wait()


def _call(x, wqkv, wo, wr, gw, wg, wu, wd):
    hbm = pl.BlockSpec(memory_space=pltpu.MemorySpace.HBM)
    return pl.pallas_call(
        _body,
        out_shape=jax.ShapeDtypeStruct((S, D), BF16),
        in_specs=[hbm] * 8,
        out_specs=hbm,
        scratch_shapes=[
            pltpu.VMEM((S, D), BF16),
            pltpu.VMEM((3, D, D), BF16),
            pltpu.VMEM((2, NT, D // 2, 128), jnp.uint32),
            pltpu.VMEM((3, D // 2, D), jnp.uint32),
            pltpu.VMEM((D, D), BF16),
            pltpu.VMEM((D // 2, D), jnp.uint32),
            pltpu.VMEM((F, D), BF16),
            pltpu.VMEM((F, D), BF16),
            pltpu.VMEM((F, D), BF16),
            pltpu.VMEM((D,), BF16),
            pltpu.VMEM((D,), BF16),
            pltpu.VMEM((2, NT, T, 128), F32),
            pltpu.VMEM((NT, S + 2 * HALO, 128), F32),
            pltpu.VMEM((NT, S + 2 * HALO, 128), F32),
            pltpu.VMEM((T + S // 2, D), jnp.uint32),
            pltpu.VMEM((T, D), jnp.uint32),
            pltpu.VMEM((S, D), F32),
            pltpu.VMEM((S, D), BF16),
            pltpu.SemaphoreType.DMA((9,)),
            pltpu.SemaphoreType.DMA((NB,)),
            pltpu.SemaphoreType.DMA((NB,)),
            pltpu.SemaphoreType.DMA((2,)),
        ],
        compiler_params=pltpu.CompilerParams(
            vmem_limit_bytes=100 * 1024 * 1024,
            flags={"XLA_TPU_EVENLY_DISTRIBUTE_CRITICAL_NODES": True}),
    )(x, wqkv, wo, wr, gw, wg, wu, wd)


@jax.jit
def pallas_gated_mix__sliding_local_dilated__moe_arch_mod__prompt_kernel(
        A_x, A_wqkv, A_wo, B_x, B_w_r, B_w_gate, B_w_up, B_w_down, gate_w):
    out = _call(A_x.reshape(S, D), A_wqkv, A_wo, B_w_r, gate_w,
                B_w_gate.T, B_w_up.T, B_w_down)
    return out.reshape(1, S, D)
```
